```python
import os as _os
_os.environ.setdefault("JAX_PLATFORMS", "cpu")
import jax
import jax.numpy as jnp

def _softmax(x, axis=-1):
    return jax.nn.softmax(x, axis=axis)
def _gelu(x):
    return jax.nn.gelu(x, approximate=True)
def _silu(x):
    return jax.nn.silu(x)
def _sigmoid(x):
    return jax.nn.sigmoid(x)
def _layernorm(x, axis=-1, eps=1e-5):
    m = jnp.mean(x, axis=axis, keepdims=True)
    v = jnp.var(x, axis=axis, keepdims=True)
    return (x - m) / jnp.sqrt(v + eps)
def _scatter_add(tgt, idx, src, axis=0):
    return tgt.at[idx].add(src)
def _segment_sum(src, seg, n):
    return jax.ops.segment_sum(src, seg, n)
class _Rng:
    def __init__(self, key):
        self._k = key
    def _next(self):
        self._k, sub = jax.random.split(self._k)
        return sub
    def normal(self, shape):
        return jax.random.normal(self._next(), shape, dtype=jnp.bfloat16)
    def randint(self, lo, hi, shape):
        return jax.random.randint(self._next(), shape, lo, hi, dtype=jnp.int32)
    def uniform(self, shape, lo=0.0, hi=1.0):
        return jax.random.uniform(self._next(), shape, jnp.bfloat16, lo, hi)
    def permutation(self, n):
        return jax.random.permutation(self._next(), n)


kernel_name = 'standalone__sliding_local_fixed_window__prompt'

def setup_inputs():
    _rng = _Rng(jax.random.key(int.from_bytes(__import__("os").urandom(4), "little")))
    _w = (lambda a: (lambda t: t.astype(jnp.bfloat16) if jnp.issubdtype(t.dtype, jnp.floating) else t)(jnp.asarray(a)))
    B, H, S, D = 1, 32, 2048, 128
    return {
        "q": _w((lambda *s: _rng.normal(s) * 0.4)(B, H, S, D)),
        "k": _w((lambda *s: _rng.normal(s) * 0.4)(B, H, S, D)),
        "v": _w((lambda *s: _rng.normal(s) * 0.05)(B, H, S, D)),
    }

def reference(q, k, v):
    B, H, S, D = q.shape
    w = 32
    pos = jnp.arange(S)
    rel = pos[:, None] - pos[None, :]
    mask = (rel >= 0) & (rel < w)
    scores = jnp.einsum("bhqd,bhkd->bhqk", q, k) * (D ** -0.5)
    scores = jnp.where(mask[None, None], scores, (lambda x, dt: x.astype(dt))(jnp.array(-1e9), q.dtype))
    p = _softmax(scores, axis=-1)
    return jnp.einsum("bhqk,bhkd->bhqd", p, v)
```

```python
import functools, math, os
import jax
import jax.numpy as jnp
from jax.experimental import pallas as pl
from jax.experimental.pallas import tpu as pltpu

W = 32
TK = 128
TQ = TK - W
NEG = -1e30
RC = int(os.environ.get('RC', '128'))
WC = int(os.environ.get('WC', '256'))
DEPTH = int(os.environ.get('DEPTH', '3'))
W0 = int(os.environ.get('W0', '4'))
WH = int(os.environ.get('WH', '31'))

def _attn_block(q, k, v, cap, c):
    s = jax.lax.dot_general(q, k, (((1,), (1,)), ((), ())), preferred_element_type=jnp.float32)
    s = jnp.minimum(s, cap)
    m = jnp.max(s, axis=-1, keepdims=True)
    p = jnp.exp2((s - m) * c)
    l = jnp.sum(p, axis=-1, keepdims=True)
    o = jnp.dot(p.astype(jnp.bfloat16), v, preferred_element_type=jnp.float32)
    return (o * pl.reciprocal(l, approx=True)).astype(jnp.bfloat16)

def _kernel(q_hbm, k_hbm, v_hbm, o_hbm, buf, ob, isem, osem, *, H, S, D):
    c = (D ** -0.5) * math.log2(math.e)
    srcs = (q_hbm, k_hbm, v_hbm)

    def issue_reads(h):
        for ch in range(S // RC):
            for a in range(3):
                pltpu.make_async_copy(srcs[a].at[h, pl.ds(ch * RC, RC)], buf.at[h, a, pl.ds(ch * RC, RC)], isem.at[h]).start(priority=ch % 2)

    def wait_reads(h):
        pltpu.make_async_copy(buf.at[h], buf.at[h], isem.at[h]).wait()

    def issue_writes(h):
        for ch in range(S // WC):
            pltpu.make_async_copy(ob.at[h, pl.ds(ch * WC, WC)], o_hbm.at[h, pl.ds(ch * WC, WC)], osem.at[0]).start(priority=ch % 2)

    def compute(h):
        b32 = buf.bitcast(jnp.uint32)
        def ld(a, start, n):
            return pltpu.bitcast(b32[h, a, pl.ds(start // 2, n // 2), :], jnp.bfloat16)
        row = jax.lax.broadcasted_iota(jnp.int32, (TK, TK), 0)
        col = jax.lax.broadcasted_iota(jnp.int32, (TK, TK), 1)
        rel0 = row - col
        cap0 = jnp.where((rel0 >= 0) & (rel0 < W), jnp.inf, NEG).astype(jnp.float32)
        rel1 = rel0[:TQ] + W
        cap1 = jnp.where((rel1 >= 0) & (rel1 < W), jnp.inf, NEG).astype(jnp.float32)
        ob[h, 0:TK, :] = _attn_block(ld(0, 0, TK), ld(1, 0, TK), ld(2, 0, TK), cap0, c)
        for j in range((S - TK) // TQ):
            qs = TK + j * TQ
            ks = TQ + j * TQ
            ob[h, qs:qs + TQ, :] = _attn_block(ld(0, qs, TQ), ld(1, ks, TK), ld(2, ks, TK), cap1, c)

    def pro(h, carry):
        issue_reads(h)
        return carry
    jax.lax.fori_loop(0, DEPTH, pro, 0)

    def wr(h, carry):
        issue_writes(h)
        return carry

    def body(h, carry):
        wait_reads(h)
        @pl.when(h + DEPTH < H)
        def _():
            issue_reads(h + DEPTH)
        @pl.when(h == WH)
        def _():
            jax.lax.fori_loop(0, W0, wr, 0)
        compute(h)
        return carry
    jax.lax.fori_loop(0, H, body, 0)
    jax.lax.fori_loop(W0, H, wr, 0)
    pltpu.make_async_copy(ob, ob, osem.at[0]).wait()

@jax.jit
def pallas_standalone__sliding_local_fixed_window__prompt_kernel(q, k, v):
    B, H, S, D = q.shape
    BH = B * H
    q3 = q.reshape(BH, S, D); k3 = k.reshape(BH, S, D); v3 = v.reshape(BH, S, D)
    spec = pl.BlockSpec(memory_space=pl.ANY)
    out = pl.pallas_call(
        functools.partial(_kernel, H=BH, S=S, D=D),
        in_specs=[spec, spec, spec],
        out_specs=spec,
        out_shape=jax.ShapeDtypeStruct((BH, S, D), q.dtype),
        scratch_shapes=[pltpu.VMEM((BH, 3, S, D), q.dtype), pltpu.VMEM((BH, S, D), q.dtype),
                        pltpu.SemaphoreType.DMA((BH,)), pltpu.SemaphoreType.DMA((1,))],
        compiler_params=pltpu.CompilerParams(vmem_limit_bytes=100 * 1024 * 1024,
                                             disable_bounds_checks=True, disable_semaphore_checks=True),
    )(q3, k3, v3)
    return out.reshape(B, H, S, D)
```

```python
import functools
import math

import jax
import jax.numpy as jnp
from jax.experimental import pallas as pl
from jax.experimental.pallas import tpu as pltpu

WINDOW = 32
TK = 128
TQ = TK - WINDOW
MASKED = -1e30

READ_ROWS = (144,) * 6 + (160,) * 2 + (144,) * 6
LOOKAHEAD = 3
TAIL_PAIRS = 4
DEFER = 2
WRITE_ROWS = 128
HEAD_STRIDE = 4


def _attn_tile(q, k, v, mask, c):
    s = jax.lax.dot_general(q, k, (((1,), (1,)), ((), ())),
                            preferred_element_type=jnp.float32)
    s = jnp.where(mask, s, MASKED)
    m = jnp.max(s, axis=-1, keepdims=True)
    p = jnp.exp2((s - m) * c)
    l = jnp.sum(p, axis=-1, keepdims=True)
    o = jnp.dot(p.astype(v.dtype), v, preferred_element_type=jnp.float32)
    return (o / l).astype(v.dtype)


def _kernel(q_hbm, k_hbm, v_hbm, o_hbm, buf, ob, isem, osem, *, H, S, D):
    c = (D ** -0.5) * math.log2(math.e)
    srcs = (q_hbm, k_hbm, v_hbm)
    starts = [sum(READ_ROWS[:i]) for i in range(len(READ_ROWS))]
    npairs = len(READ_ROWS) // 2
    split_row = starts[2 * (npairs - TAIL_PAIRS)]
    ring = LOOKAHEAD + 1
    tail_sem = isem.at[ring]

    def head_sem(h):
        return isem.at[h % ring]

    def issue_reads(h, last=False):
        n = 0
        for j in range(npairs):
            sem = tail_sem if (last and j >= npairs - TAIL_PAIRS) else head_sem(h)
            for a in range(3):
                for i in (2 * j, 2 * j + 1):
                    rows = pl.ds(starts[i], READ_ROWS[i])
                    pltpu.make_async_copy(srcs[a].at[h, rows], buf.at[h, a, rows],
                                          sem).start(priority=n % 2)
                    n += 1

    def wait_filled(region, sem):
        pltpu.make_async_copy(region, region, sem).wait()

    def issue_writes(j):
        for p in range(S // WRITE_ROWS):
            rows = pl.ds(p * WRITE_ROWS, WRITE_ROWS)
            pltpu.make_async_copy(ob.at[:, j, rows], o_hbm.at[:, j, rows],
                                  osem.at[0]).start()

    def compute(h):
        hi = h // HEAD_STRIDE
        hj = h % HEAD_STRIDE
        rel = (jax.lax.broadcasted_iota(jnp.int32, (TK, TK), 0)
               - jax.lax.broadcasted_iota(jnp.int32, (TK, TK), 1))
        mask0 = (rel >= 0) & (rel < WINDOW)
        rel1 = rel[:TQ] + WINDOW
        mask1 = (rel1 >= 0) & (rel1 < WINDOW)
        ob[hi, hj, 0:TK, :] = _attn_tile(buf[h, 0, 0:TK, :], buf[h, 1, 0:TK, :],
                                         buf[h, 2, 0:TK, :], mask0, c)
        for t in range((S - TK) // TQ):
            qs = TK + t * TQ
            ks = qs - WINDOW
            ob[hi, hj, qs:qs + TQ, :] = _attn_tile(
                buf[h, 0, qs:qs + TQ, :], buf[h, 1, ks:ks + TK, :],
                buf[h, 2, ks:ks + TK, :], mask1, c)

    for h in range(LOOKAHEAD):
        issue_reads(h)

    def body(h, carry):
        @pl.when(h + LOOKAHEAD < H - 1)
        def _():
            issue_reads(h + LOOKAHEAD)

        @pl.when(h + LOOKAHEAD == H - 1)
        def _():
            issue_reads(H - 1, last=True)

        @pl.when(h < H - DEFER)
        def _():
            wait_filled(buf.at[h], head_sem(h))

        @pl.when(h == H - DEFER)
        def _():
            for hh in range(H - DEFER, H - 1):
                wait_filled(buf.at[hh], head_sem(hh))
            wait_filled(buf.at[H - 1, :, pl.ds(0, split_row)], head_sem(H - 1))
            for j in range(HEAD_STRIDE - DEFER):
                issue_writes(j)
            wait_filled(buf.at[H - 1, :, pl.ds(split_row, S - split_row)], tail_sem)

        compute(h)
        return carry

    jax.lax.fori_loop(0, H, body, 0)
    for j in range(HEAD_STRIDE - DEFER, HEAD_STRIDE):
        issue_writes(j)
    pltpu.make_async_copy(ob, o_hbm, osem.at[0]).wait()


@jax.jit
def pallas_standalone__sliding_local_fixed_window__prompt_kernel(
    q: jax.Array,
    k: jax.Array,
    v: jax.Array,
):
    B, H, S, D = q.shape
    BH = B * H
    assert sum(READ_ROWS) == S and (S - TK) % TQ == 0 and S % WRITE_ROWS == 0
    assert BH % HEAD_STRIDE == 0 and BH > LOOKAHEAD + DEFER and DEFER < HEAD_STRIDE
    out_view = (BH // HEAD_STRIDE, HEAD_STRIDE, S, D)
    any_spec = pl.BlockSpec(memory_space=pl.ANY)
    out = pl.pallas_call(
        functools.partial(_kernel, H=BH, S=S, D=D),
        in_specs=[any_spec, any_spec, any_spec],
        out_specs=any_spec,
        out_shape=jax.ShapeDtypeStruct(out_view, q.dtype),
        scratch_shapes=[
            pltpu.VMEM((BH, 3, S, D), q.dtype),
            pltpu.VMEM(out_view, q.dtype),
            pltpu.SemaphoreType.DMA((LOOKAHEAD + 2,)),
            pltpu.SemaphoreType.DMA((1,)),
        ],
        compiler_params=pltpu.CompilerParams(
            vmem_limit_bytes=100 * 1024 * 1024,
            disable_bounds_checks=True,
            disable_semaphore_checks=True,
        ),
    )(q.reshape(BH, S, D), k.reshape(BH, S, D), v.reshape(BH, S, D))
    return out.reshape(B, H, S, D)
```

```python
import functools
import math

import jax
import jax.numpy as jnp
from jax.experimental import pallas as pl
from jax.experimental.pallas import tpu as pltpu

WINDOW = 32
TK = 128
TQ = TK - WINDOW
MASKED = -1e30

NG = 4
CHUNK = 128
SHIFT = 104
HEAD_ORDER = (0, 4, 1, 5, 2, 6, 3, 7)
LAG = 10
TAIL = 3
TRANS = 22


def _attn_tile(q, k, v, mask, c):
    s = jax.lax.dot_general(q, k, (((1,), (1,)), ((), ())),
                            preferred_element_type=jnp.float32)
    s = jnp.where(mask, s, MASKED)
    m = jnp.max(s, axis=-1, keepdims=True)
    p = jnp.exp2((s - m) * c)
    l = jnp.sum(p, axis=-1, keepdims=True)
    o = jnp.dot(p.astype(v.dtype), v, preferred_element_type=jnp.float32)
    return (o / l).astype(v.dtype)


def _kernel(q_hbm, k_hbm, v_hbm, o_hbm, buf, ob, isem, osem, *, GH, S, D):
    c = (D ** -0.5) * math.log2(math.e)
    srcs = (q_hbm, k_hbm, v_hbm)
    H = NG * GH
    last0 = H - GH
    assert LAG > GH and TRANS + LAG >= H - 1 and last0 - GH < TRANS < last0

    full = [(SHIFT + n * CHUNK, CHUNK) for n in range((S - SHIFT) // CHUNK)]
    end = full[-1][0] + CHUNK
    chunks = [(0, SHIFT), (end, S - end)] + full
    rows = [(a, st, sz) for a in range(3) for st, sz in chunks]
    nrows = len(rows)
    bounds = [(u * nrows) // GH for u in range(GH + 1)]
    tail_lo = full[-TAIL][0]

    def issue_read_slice(j, u):
        tail_idx = jnp.where(j == NG - 1, NG, j)
        for r in range(bounds[u], bounds[u + 1]):
            a, st, sz = rows[r]
            sem = isem.at[tail_idx] if r >= nrows - TAIL else isem.at[j]
            for n, i in enumerate(HEAD_ORDER):
                pltpu.make_async_copy(srcs[a].at[i, j, pl.ds(st, sz)],
                                      buf.at[j, a, i, pl.ds(st, sz)],
                                      sem).start(priority=n % 2)

    def wait_filled(region, sem):
        pltpu.make_async_copy(region, region, sem).wait()

    def issue_writes(j):
        for p in range(S // CHUNK):
            r = pl.ds(p * CHUNK, CHUNK)
            pltpu.make_async_copy(ob.at[:, j, r], o_hbm.at[:, j, r], osem.at[0]).start()

    def compute(j, i):
        rel = (jax.lax.broadcasted_iota(jnp.int32, (TK, TK), 0)
               - jax.lax.broadcasted_iota(jnp.int32, (TK, TK), 1))
        mask0 = (rel >= 0) & (rel < WINDOW)
        rel1 = rel[:TQ] + WINDOW
        mask1 = (rel1 >= 0) & (rel1 < WINDOW)
        ob[i, j, 0:TK, :] = _attn_tile(buf[j, 0, i, 0:TK, :], buf[j, 1, i, 0:TK, :],
                                       buf[j, 2, i, 0:TK, :], mask0, c)
        for t in range((S - TK) // TQ):
            qs = TK + t * TQ
            ks = qs - WINDOW
            ob[i, j, qs:qs + TQ, :] = _attn_tile(
                buf[j, 0, i, qs:qs + TQ, :], buf[j, 1, i, ks:ks + TK, :],
                buf[j, 2, i, ks:ks + TK, :], mask1, c)

    def body(s, carry):
        @pl.when(s < H)
        def _():
            for u in range(GH):
                @pl.when(s % GH == u)
                def _():
                    issue_read_slice(s // GH, u)

        t = s - LAG

        @pl.when(t >= 0)
        def _():
            j = t // GH
            i = t % GH

            @pl.when((i == 0) & (t < last0))
            def _():
                wait_filled(buf.at[j], isem.at[j])

            @pl.when(t == TRANS)
            def _():
                g = NG - 1
                wait_filled(buf.at[g, 0:2], isem.at[g])
                wait_filled(buf.at[g, 2, :, pl.ds(0, tail_lo)], isem.at[g])
                wait_filled(buf.at[g, 2, :, pl.ds(end, S - end)], isem.at[g])
                for jj in range(NG - 2):
                    issue_writes(jj)
                wait_filled(buf.at[g, 2, :, pl.ds(tail_lo, end - tail_lo)], isem.at[NG])

            @pl.when(t == last0)
            def _():
                issue_writes(NG - 2)

            compute(j, i)

        return carry

    jax.lax.fori_loop(0, H + LAG, body, 0)
    issue_writes(NG - 1)
    pltpu.make_async_copy(ob, o_hbm, osem.at[0]).wait()


@jax.jit
def pallas_standalone__sliding_local_fixed_window__prompt_kernel(
    q: jax.Array,
    k: jax.Array,
    v: jax.Array,
):
    B, H, S, D = q.shape
    GH = B * H // NG
    assert GH * NG == B * H and GH == len(HEAD_ORDER)
    assert (S - TK) % TQ == 0 and S % CHUNK == 0
    view = (GH, NG, S, D)
    any_spec = pl.BlockSpec(memory_space=pl.ANY)
    out = pl.pallas_call(
        functools.partial(_kernel, GH=GH, S=S, D=D),
        in_specs=[any_spec, any_spec, any_spec],
        out_specs=any_spec,
        out_shape=jax.ShapeDtypeStruct(view, q.dtype),
        scratch_shapes=[
            pltpu.VMEM((NG, 3, GH, S, D), q.dtype),
            pltpu.VMEM(view, q.dtype),
            pltpu.SemaphoreType.DMA((NG + 1,)),
            pltpu.SemaphoreType.DMA((1,)),
        ],
        compiler_params=pltpu.CompilerParams(
            vmem_limit_bytes=100 * 1024 * 1024,
            disable_bounds_checks=True,
            disable_semaphore_checks=True,
        ),
    )(q.reshape(view), k.reshape(view), v.reshape(view))
    return out.reshape(B, H, S, D)
```

```python
import functools
import math

import jax
import jax.numpy as jnp
from jax.experimental import pallas as pl
from jax.experimental.pallas import tpu as pltpu

WINDOW = 32
TK = 128
TQ = TK - WINDOW
MASKED = -1e30

NG = 4
CHUNK = 128
SHIFT = 104
HEAD_ORDER = (0, 4, 1, 5, 2, 6, 3, 7)
LAG = 10
TAIL = 3
TRANS = 22
SPLIT = 4


def _attn_tile(q, k, v, mask, c):
    s = jax.lax.dot_general(q, k, (((1,), (1,)), ((), ())),
                            preferred_element_type=jnp.float32)
    s = jnp.where(mask, s, MASKED)
    m = jnp.max(s, axis=-1, keepdims=True)
    p = jnp.exp2((s - m) * c)
    l = jnp.sum(p, axis=-1, keepdims=True)
    o = jnp.dot(p.astype(v.dtype), v, preferred_element_type=jnp.float32)
    return (o / l).astype(v.dtype)


def _kernel(q_hbm, k_hbm, v_hbm, o_hbm, buf, ob, isem, osem, *, GH, S, D):
    c = (D ** -0.5) * math.log2(math.e)
    srcs = (q_hbm, k_hbm, v_hbm)
    H = NG * GH
    last0 = H - GH
    assert LAG > GH and TRANS + LAG >= H - 1 and last0 - GH < TRANS < last0
    assert 0 < SPLIT < GH

    full = [(SHIFT + n * CHUNK, CHUNK) for n in range((S - SHIFT) // CHUNK)]
    end = full[-1][0] + CHUNK
    chunks = [(0, SHIFT), (end, S - end)] + full
    rows = [(a, st, sz) for a in range(3) for st, sz in chunks]
    nrows = len(rows)
    bounds = [(u * nrows) // GH for u in range(GH + 1)]
    tail_lo = full[-TAIL][0]

    def issue_read_slice(j, u):
        tail_idx = jnp.where(j == NG - 1, NG, j)
        for r in range(bounds[u], bounds[u + 1]):
            a, st, sz = rows[r]
            sem = isem.at[tail_idx] if r >= nrows - TAIL else isem.at[j]
            for n, i in enumerate(HEAD_ORDER):
                pltpu.make_async_copy(srcs[a].at[i, j, pl.ds(st, sz)],
                                      buf.at[j, a, i, pl.ds(st, sz)],
                                      sem).start(priority=n % 2)

    def wait_filled(region, sem):
        pltpu.make_async_copy(region, region, sem).wait()

    def issue_writes(j, i0=0, ni=GH):
        heads = pl.ds(i0, ni)
        for p in range(S // CHUNK):
            r = pl.ds(p * CHUNK, CHUNK)
            pltpu.make_async_copy(ob.at[heads, j, r], o_hbm.at[heads, j, r],
                                  osem.at[0]).start()

    def compute(j, i):
        rel = (jax.lax.broadcasted_iota(jnp.int32, (TK, TK), 0)
               - jax.lax.broadcasted_iota(jnp.int32, (TK, TK), 1))
        mask0 = (rel >= 0) & (rel < WINDOW)
        rel1 = rel[:TQ] + WINDOW
        mask1 = (rel1 >= 0) & (rel1 < WINDOW)
        ob[i, j, 0:TK, :] = _attn_tile(buf[j, 0, i, 0:TK, :], buf[j, 1, i, 0:TK, :],
                                       buf[j, 2, i, 0:TK, :], mask0, c)
        for t in range((S - TK) // TQ):
            qs = TK + t * TQ
            ks = qs - WINDOW
            ob[i, j, qs:qs + TQ, :] = _attn_tile(
                buf[j, 0, i, qs:qs + TQ, :], buf[j, 1, i, ks:ks + TK, :],
                buf[j, 2, i, ks:ks + TK, :], mask1, c)

    def body(s, carry):
        @pl.when(s < H)
        def _():
            for u in range(GH):
                @pl.when(s % GH == u)
                def _():
                    issue_read_slice(s // GH, u)

        t = s - LAG

        @pl.when(t >= 0)
        def _():
            j = t // GH
            i = t % GH

            @pl.when((i == 0) & (t < last0))
            def _():
                wait_filled(buf.at[j], isem.at[j])

            @pl.when(t == TRANS)
            def _():
                g = NG - 1
                wait_filled(buf.at[g, 0:2], isem.at[g])
                wait_filled(buf.at[g, 2, :, pl.ds(0, tail_lo)], isem.at[g])
                wait_filled(buf.at[g, 2, :, pl.ds(end, S - end)], isem.at[g])
                for jj in range(NG - 2):
                    issue_writes(jj)
                wait_filled(buf.at[g, 2, :, pl.ds(tail_lo, end - tail_lo)], isem.at[NG])

            @pl.when(t == last0)
            def _():
                issue_writes(NG - 2)

            @pl.when(t == last0 + SPLIT)
            def _():
                issue_writes(NG - 1, 0, SPLIT)

            compute(j, i)

        return carry

    jax.lax.fori_loop(0, H + LAG, body, 0)
    issue_writes(NG - 1, SPLIT, GH - SPLIT)
    pltpu.make_async_copy(ob, o_hbm, osem.at[0]).wait()


@jax.jit
def pallas_standalone__sliding_local_fixed_window__prompt_kernel(
    q: jax.Array,
    k: jax.Array,
    v: jax.Array,
):
    B, H, S, D = q.shape
    GH = B * H // NG
    assert GH * NG == B * H and GH == len(HEAD_ORDER)
    assert (S - TK) % TQ == 0 and S % CHUNK == 0
    view = (GH, NG, S, D)
    any_spec = pl.BlockSpec(memory_space=pl.ANY)
    out = pl.pallas_call(
        functools.partial(_kernel, GH=GH, S=S, D=D),
        in_specs=[any_spec, any_spec, any_spec],
        out_specs=any_spec,
        out_shape=jax.ShapeDtypeStruct(view, q.dtype),
        scratch_shapes=[
            pltpu.VMEM((NG, 3, GH, S, D), q.dtype),
            pltpu.VMEM(view, q.dtype),
            pltpu.SemaphoreType.DMA((NG + 1,)),
            pltpu.SemaphoreType.DMA((1,)),
        ],
        compiler_params=pltpu.CompilerParams(
            vmem_limit_bytes=100 * 1024 * 1024,
            disable_bounds_checks=True,
            disable_semaphore_checks=True,
        ),
    )(q.reshape(view), k.reshape(view), v.reshape(view))
    return out.reshape(B, H, S, D)
```
